```python
import jax
import jax.numpy as jnp

def _softmax(x, axis=-1):
    return jax.nn.softmax(x, axis=axis)
def _gelu(x):
    return jax.nn.gelu(x, approximate=True)
def _silu(x):
    return jax.nn.silu(x)
def _sigmoid(x):
    return jax.nn.sigmoid(x)
def _layernorm(x, axis=-1, eps=1e-5):
    m = jnp.mean(x, axis=axis, keepdims=True)
    v = jnp.var(x, axis=axis, keepdims=True)
    return (x - m) / jnp.sqrt(v + eps)
def _scatter_add(tgt, idx, src, axis=0):
    return tgt.at[idx].add(src)
def _segment_sum(src, seg, n):
    return jax.ops.segment_sum(src, seg, n)
class _Rng:
    def __init__(self, key):
        self._k = key
    def _next(self):
        self._k, sub = jax.random.split(self._k)
        return sub
    def normal(self, shape):
        return jax.random.normal(self._next(), shape, dtype=jnp.bfloat16)
    def randint(self, lo, hi, shape):
        return jax.random.randint(self._next(), shape, lo, hi, dtype=jnp.int32)
    def uniform(self, shape, lo=0.0, hi=1.0):
        return jax.random.uniform(self._next(), shape, jnp.bfloat16, lo, hi)
    def permutation(self, n):
        return jax.random.permutation(self._next(), n)


kernel_name = 'parallel_sum__sliding_local_dilated__mixer_channel_mlp__prompt'

def _fwd_setup_inputs():
    _rng = _Rng(jax.random.key(int.from_bytes(__import__("os").urandom(4), "little")))
    _w = (lambda a: (lambda t: t.astype(jnp.bfloat16) if jnp.issubdtype(t.dtype, jnp.floating) else t)(jnp.asarray(a)))
    def _A_setup():
        B, S, D = 1, 2048, 576
        return {
            "x": _w((lambda *s: _rng.normal(s) * 0.05)(B, S, D)),
            "wqkv": _w((lambda *s: _rng.normal(s) * 0.05)(D, 3 * D)),
            "wo": _w((lambda *s: _rng.normal(s) * 0.05)(D, D)),
        }
    _A_in = _A_setup()

    def _B_setup():
        B, S, D, F = 1, 2048, 576, 4608
        return {
            "x": _w((lambda *s: _rng.normal(s) * 0.05)(B, S, D)),
            "w1": _w((lambda *s: _rng.normal(s) * 0.05)(D, F) * (D ** -0.5)),
            "b1": _w((lambda *s: _rng.normal(s) * 0.05)(F)),
            "w2": _w((lambda *s: _rng.normal(s) * 0.05)(F, D) * (F ** -0.5)),
            "b2": _w((lambda *s: _rng.normal(s) * 0.05)(D)),
        }
    _B_in = _B_setup()

    return {
        "A_x": _A_in["x"],
        "A_wqkv": _A_in["wqkv"],
        "A_wo": _A_in["wo"],
        "B_x": _B_in["x"],
        "B_w1": _B_in["w1"],
        "B_b1": _B_in["b1"],
        "B_w2": _B_in["w2"],
        "B_b2": _B_in["b2"],
    }

def _fwd_reference(A_x, A_wqkv, A_wo, B_x, B_w1, B_b1, B_w2, B_b2):
    def _A_ref(x, wqkv, wo):
        B, S, D = x.shape
        H = 32; Dh = D // H
        W, dil = 8, 2
        qkv = (lambda x, *d: x.transpose(*d))((x @ wqkv).reshape(B, S, 3, H, Dh), 2, 0, 3, 1, 4)
        q, k, v = qkv[0], qkv[1], qkv[2]
        scale = Dh ** -0.5
        pos = jnp.arange(S)
        off = jnp.arange(W) * dil
        idx = pos[:, None] - off[None, :]
        mask = idx >= 0
        idx_c = jnp.where(mask, idx, 0).reshape(-1)
        kg = k[:, :, idx_c, :].reshape(B, H, S, W, Dh)
        vg = v[:, :, idx_c, :].reshape(B, H, S, W, Dh)
        logits = jnp.einsum("bhsd,bhswd->bhsw", q, kg) * scale
        logits = jnp.where(mask[None, None, :, :], logits, -1e9)
        attn = _softmax(logits, axis=-1)
        o = jnp.einsum("bhsw,bhswd->bhsd", attn, vg)
        return (lambda x, *d: x.transpose(*d))(o, 0, 2, 1, 3).reshape(B, S, D) @ wo

    def _B_ref(x, w1, b1, w2, b2):
        y = _layernorm(x, axis=-1)
        h = _gelu(jnp.einsum("bsd,df->bsf", y, w1) + b1)
        return jnp.einsum("bsf,fd->bsd", h, w2) + b2

    x = A_x
    xn = _layernorm(x, axis=-1)
    return x + _A_ref(xn, A_wqkv, A_wo) + _B_ref(xn, B_w1, B_b1, B_w2, B_b2)


def setup_inputs():
    _inp = _fwd_setup_inputs()
    _gk = jax.random.fold_in(jax.random.key(int.from_bytes(__import__("os").urandom(4), "little")), 2**31 - 1)
    _shapes = [[1, 2048, 576]]
    _dtypes = ['bfloat16']
    _gks = jax.random.split(_gk, len(_shapes))
    _gs = [jax.random.normal(k, s, dtype=jnp.dtype(d)) * 0.05 for k, s, d in zip(_gks, _shapes, _dtypes)]
    _inp["grad_out"] = _gs[0]
    return _inp

def reference(A_x, A_wqkv, A_wo, B_w1, B_b1, B_w2, B_b2, B_x, grad_out):
    _const = dict(B_x=B_x)
    def _f(*_d):
        return _fwd_reference(**{'A_x': _d[0], 'A_wqkv': _d[1], 'A_wo': _d[2], 'B_w1': _d[3], 'B_b1': _d[4], 'B_w2': _d[5], 'B_b2': _d[6], **_const})
    _out, _vjp = jax.vjp(_f, A_x, A_wqkv, A_wo, B_w1, B_b1, B_w2, B_b2)
    _grads = _vjp(grad_out)
    _out0 = jnp.asarray(_out)
    return (_out0, *[jnp.asarray(_g) for _g in _grads])
```

```python
import jax
import jax.numpy as jnp
from jax import lax
import jax.experimental.pallas as pl
import jax.experimental.pallas.tpu as pltpu

BF16 = jnp.bfloat16
F32 = jnp.float32

S, D, F = 2048, 576, 4608
DP = 640
DH, WIN, DIL = 18, 8, 2
LANES = 128
NT_ = S // LANES
FC = 512
NF = F // FC
PROWS = 72
NP = D // PROWS
RC = 64
EPS = 1e-5
SCALE = DH ** -0.5
C0 = 0.7978845608028654
C1 = C0 * 0.044715

NN = (((1,), (0,)), ((), ()))
NT = (((1,), (1,)), ((), ()))
TN = (((0,), (0,)), ((), ()))


def _dot(a, b, dn=NN):
    return lax.dot_general(a, b, dn, preferred_element_type=F32)


def _gelu_pair(x):
    x2 = x * x
    t = jnp.tanh(x * (C0 + C1 * x2))
    a = 0.5 + 0.5 * t
    h = x * a
    gp = a + (h * (1.0 - t)) * (C0 + (3.0 * C1) * x2)
    return h, gp


def _colmean(a):
    return jnp.sum(a, axis=0, keepdims=True) * (1.0 / D)


def _layernorm_t(u):
    c = u - _colmean(u)
    r = lax.rsqrt(_colmean(c * c) + EPS)
    return c * r, r


def _layernorm_bwd_t(dy, y, r):
    return r * (dy - _colmean(dy) - y * _colmean(dy * y))


def _attention_piece(p, qkv_ref, do_ref, o_ref, dqkv_ref):
    base = p * PROWS
    lane = lax.broadcasted_iota(jnp.int32, (8, LANES), 1)
    even = (lax.broadcasted_iota(jnp.int32, (8, LANES), 0) & 1) == 0

    def rows(off, i):
        return pl.ds(base + off + i, 8, stride=9)

    def fold(a):
        return a + jnp.where(even, pltpu.roll(a, 7, 0), pltpu.roll(a, 1, 0))

    nd = DH // 2
    rk_prev = rv_prev = None
    uk_prev = uv_prev = None
    dk_prev = dv_prev = None
    for t in range(NT_):
        q = [qkv_ref[t, rows(0, i), :] for i in range(nd)]
        k = [qkv_ref[t, rows(D, i), :] for i in range(nd)]
        v = [qkv_ref[t, rows(2 * D, i), :] for i in range(nd)]
        do = [do_ref[t, rows(0, i), :] for i in range(nd)]
        rk = [[pltpu.roll(k[i], DIL * w, 1) if w else None for w in range(WIN)] for i in range(nd)]
        rv = [[pltpu.roll(v[i], DIL * w, 1) if w else None for w in range(WIN)] for i in range(nd)]
        if t == 0:
            k0 = [jnp.broadcast_to(k[i][:, 0:1], (8, LANES)) for i in range(nd)]
            v0 = [jnp.broadcast_to(v[i][:, 0:1], (8, LANES)) for i in range(nd)]
            rk_prev = [[k0[i]] * WIN for i in range(nd)]
            rv_prev = [[v0[i]] * WIN for i in range(nd)]
        ks = [[jnp.where(lane >= DIL * w, rk[i][w], rk_prev[i][w]) if w else k[i]
               for w in range(WIN)] for i in range(nd)]
        vs = [[jnp.where(lane >= DIL * w, rv[i][w], rv_prev[i][w]) if w else v[i]
               for w in range(WIN)] for i in range(nd)]
        rk_prev, rv_prev = rk, rv

        lg, da = [], []
        for w in range(WIN):
            a = q[0] * ks[0][w]
            b = do[0] * vs[0][w]
            for i in range(1, nd):
                a = a + q[i] * ks[i][w]
                b = b + do[i] * vs[i][w]
            a = fold(a) * SCALE
            if t == 0 and w:
                a = jnp.where(lane >= DIL * w, a, -1e9)
            lg.append(a)
            da.append(fold(b))
        m = lg[0]
        for w in range(1, WIN):
            m = jnp.maximum(m, lg[w])
        e = [jnp.exp(lg[w] - m) for w in range(WIN)]
        den = e[0]
        for w in range(1, WIN):
            den = den + e[w]
        inv = 1.0 / den
        pr = [e[w] * inv for w in range(WIN)]
        dsum = pr[0] * da[0]
        for w in range(1, WIN):
            dsum = dsum + pr[w] * da[w]
        dl = [(pr[w] * SCALE) * (da[w] - dsum) for w in range(WIN)]
        if t == 0:
            dl = [jnp.where(lane >= DIL * w, dl[w], 0.0) if w else dl[w] for w in range(WIN)]

        uk, uv, dk, dv = [], [], [], []
        for i in range(nd):
            o = pr[0] * vs[i][0]
            dq = dl[0] * ks[i][0]
            for w in range(1, WIN):
                o = o + pr[w] * vs[i][w]
                dq = dq + dl[w] * ks[i][w]
            o_ref[t, rows(0, i), :] = o
            dqkv_ref[t, rows(0, i), :] = dq
            tv = [pr[w] * do[i] for w in range(WIN)]
            uk.append([pltpu.roll(dl[w] * q[i], LANES - DIL * w, 1) if w else None for w in range(WIN)])
            uv.append([pltpu.roll(tv[w], LANES - DIL * w, 1) if w else None for w in range(WIN)])
            dk.append(dl[0] * q[i])
            dv0 = tv[0]
            if t == 0:
                z = jnp.where(lane < DIL, tv[1], 0.0)
                for w in range(2, WIN):
                    z = z + jnp.where(lane < DIL * w, tv[w], 0.0)
                dv0 = dv0 + jnp.where(lane == 0, jnp.sum(z, axis=1, keepdims=True), 0.0)
            dv.append(dv0)
            if t > 0:
                a, b = dk_prev[i], dv_prev[i]
                for w in range(1, WIN):
                    keep = lane < LANES - DIL * w
                    a = a + jnp.where(keep, uk_prev[i][w], uk[i][w])
                    b = b + jnp.where(keep, uv_prev[i][w], uv[i][w])
                dqkv_ref[t - 1, rows(D, i), :] = a
                dqkv_ref[t - 1, rows(2 * D, i), :] = b
        uk_prev, uv_prev, dk_prev, dv_prev = uk, uv, dk, dv
    for i in range(nd):
        a, b = dk_prev[i], dv_prev[i]
        for w in range(1, WIN):
            keep = lane < LANES - DIL * w
            a = a + jnp.where(keep, uk_prev[i][w], 0.0)
            b = b + jnp.where(keep, uv_prev[i][w], 0.0)
        dqkv_ref[NT_ - 1, rows(D, i), :] = a
        dqkv_ref[NT_ - 1, rows(2 * D, i), :] = b


def _kernel(xT_hbm, gT_hbm, wqkv_hbm, wo_hbm, w1_hbm, b1_ref, w2T_hbm, b2_ref,
            outT_hbm, dxT_hbm, gwqkv_hbm, gwo_hbm, gw1_hbm, gb1_ref, gw2T_hbm, gb2_ref,
            xT, gT, xnT, yT, y, g, wqkv, wo, w1b, w2b, g1b, g2b,
            h_s, dp_s, gp_s, out_acc, dy_acc, qkv_s, do_s, o_s, dqkv_s, oT, dqkvT,
            outb, dxb, gwqkv_b, gwo_b, sem_a, sem_in, sem_out):
    cp_x = pltpu.make_async_copy(xT_hbm, xT, sem_a.at[0])
    cp_g = pltpu.make_async_copy(gT_hbm, gT.at[pl.ds(0, D)], sem_a.at[1])
    cp_wqkv = pltpu.make_async_copy(wqkv_hbm, wqkv, sem_a.at[2])
    cp_wo = pltpu.make_async_copy(wo_hbm, wo.at[pl.ds(0, D)], sem_a.at[3])

    def w_copies(i, slot):
        cols = pl.ds(pl.multiple_of(i * FC, FC), FC)
        return (pltpu.make_async_copy(w1_hbm.at[:, cols], w1b.at[slot, pl.ds(0, D)], sem_in.at[0, slot]),
                pltpu.make_async_copy(w2T_hbm.at[:, cols], w2b.at[slot], sem_in.at[1, slot]))

    def g_copies(i, slot):
        cols = pl.ds(pl.multiple_of(i * FC, FC), FC)
        return (pltpu.make_async_copy(g1b.at[slot], gw1_hbm.at[:, cols], sem_out.at[0, slot]),
                pltpu.make_async_copy(g2b.at[slot], gw2T_hbm.at[:, cols], sem_out.at[1, slot]))

    cp_x.start()
    cp_wqkv.start()
    cp_g.start()
    cp_wo.start()
    for c in w_copies(0, 0):
        c.start()

    pad_row = lax.broadcasted_iota(jnp.int32, (DP - D, LANES), 0)
    one_row = jnp.where(pad_row == 0, 1.0, 0.0).astype(BF16)
    gT[D:, :] = jnp.zeros((DP - D, S), BF16)
    cp_x.wait()
    for t in range(NT_):
        ts = slice(t * LANES, (t + 1) * LANES)
        xn, _ = _layernorm_t(xT[:, ts].astype(F32))
        yv, _ = _layernorm_t(xn)
        xnT[:, ts] = xn.astype(BF16)
        yb = yv.astype(BF16)
        yT[:, ts] = yb
        y[ts, :] = jnp.concatenate([yb, one_row], axis=0).T
        oT[D:, ts] = one_row
    cp_wqkv.wait()
    TC = 512
    for c in range(S // TC):
        r = _dot(wqkv[...], xnT[:, c * TC:(c + 1) * TC], TN)
        for j in range(TC // LANES):
            qkv_s[c * (TC // LANES) + j] = r[:, j * LANES:(j + 1) * LANES]
    cp_g.wait()
    cp_wo.wait()
    gsum = jnp.zeros((8, DP), F32)
    for t in range(NT_):
        ts = slice(t * LANES, (t + 1) * LANES)
        gt = gT[:, ts].T
        g[ts, :] = gt
        gsum = gsum + gt.astype(F32).reshape(LANES // 8, 8, DP).sum(axis=0)
    gb2_ref[...] = jnp.sum(gsum, axis=0, keepdims=True)[:, :D].astype(BF16)
    for c in range(S // TC):
        r = _dot(wo[:D, :], gT[:D, c * TC:(c + 1) * TC])
        for j in range(TC // LANES):
            do_s[c * (TC // LANES) + j] = r[:, j * LANES:(j + 1) * LANES]
    pad_d = lax.broadcasted_iota(jnp.int32, (DP - D, D), 0)
    wo[D:, :] = jnp.where(pad_d == 0, b2_ref[...].astype(F32), 0.0).astype(BF16)
    out_acc[...] = jnp.zeros((D, S), F32)
    dy_acc[...] = jnp.zeros((D, S), F32)

    def mlp_step(i, carry):
        slot = i % 2
        for c in w_copies(i, slot):
            c.wait()

        @pl.when(i + 1 < NF)
        def _():
            for c in w_copies(i + 1, 1 - slot):
                c.start()

        @pl.when(i >= 2)
        def _():
            for c in g_copies(i - 2, slot):
                c.wait()

        pad_f = lax.broadcasted_iota(jnp.int32, (DP - D, FC), 0)
        w1b[slot, D:, :] = jnp.where(pad_f == 0, b1_ref[i].astype(F32), 0.0).astype(BF16)
        pre = _dot(y[...], w1b[slot])
        for r in range(0, S, RC):
            h, gp = _gelu_pair(pre[r:r + RC])
            h_s[r:r + RC, :] = h.astype(BF16)
            gp_s[r:r + RC, :] = gp
        dh = _dot(g[:, :D], w2b[slot])
        gb = jnp.zeros((8, FC), F32)
        for r in range(0, S, RC):
            dp = dh[r:r + RC] * gp_s[r:r + RC, :]
            dp_s[r:r + RC, :] = dp.astype(BF16)
            gb = gb + dp.reshape(RC // 8, 8, FC).sum(axis=0)
        gb1_ref[i] = jnp.sum(gb, axis=0, keepdims=True).astype(BF16)
        _attention_piece(jnp.minimum(i, NP - 1), qkv_s, do_s, o_s, dqkv_s)
        out_acc[...] += _dot(w2b[slot], h_s[...], NT)
        g2b[slot] = _dot(gT[:D, :], h_s[...]).astype(BF16)
        dy_acc[...] += _dot(w1b[slot, :D, :], dp_s[...], NT)
        g1b[slot] = _dot(yT[...], dp_s[...]).astype(BF16)
        for c in g_copies(i, slot):
            c.start()
        return carry

    lax.fori_loop(0, NF, mlp_step, 0)

    for t in range(NT_):
        ts = slice(t * LANES, (t + 1) * LANES)
        oT[:D, ts] = o_s[t].astype(BF16)
        dqkvT[:, ts] = dqkv_s[t].astype(BF16)
    for c in range(S // TC):
        dxn = _dot(wqkv[...], dqkvT[:, c * TC:(c + 1) * TC])
        for j in range(TC // LANES):
            ts = slice(c * TC + j * LANES, c * TC + (j + 1) * LANES)
            xn, r1 = _layernorm_t(xT[:, ts].astype(F32))
            yv, r2 = _layernorm_t(xn)
            d = dxn[:, j * LANES:(j + 1) * LANES] + _layernorm_bwd_t(dy_acc[:, ts], yv, r2)
            dxb[:, ts] = (gT[:D, ts].astype(F32) + _layernorm_bwd_t(d, xn, r1)).astype(BF16)
    st_dx = pltpu.make_async_copy(dxb, dxT_hbm, sem_a.at[0])
    st_dx.start()
    for c in range(S // TC):
        ts = slice(c * TC, (c + 1) * TC)
        a = _dot(wo[...], oT[:, ts], TN)
        outb[:, ts] = (a + out_acc[:, ts] + xT[:, ts].astype(F32)).astype(BF16)
    st_out = pltpu.make_async_copy(outb, outT_hbm, sem_a.at[1])
    st_out.start()
    gwqkv_b[...] = _dot(xnT[...], dqkvT[...], NT).astype(BF16)
    st_gwqkv = pltpu.make_async_copy(gwqkv_b, gwqkv_hbm, sem_a.at[2])
    st_gwqkv.start()
    gwo_b[...] = _dot(oT[:D, :], gT[:D, :], NT).astype(BF16)
    st_gwo = pltpu.make_async_copy(gwo_b, gwo_hbm, sem_a.at[3])
    st_gwo.start()
    for i in (NF - 2, NF - 1):
        for c in g_copies(i, i % 2):
            c.wait()
    st_dx.wait()
    st_out.wait()
    st_gwqkv.wait()
    st_gwo.wait()


@jax.jit
def pallas_parallel_sum__sliding_local_dilated__mixer_channel_mlp__prompt_kernel(
    A_x: jax.Array,
    A_wqkv: jax.Array,
    A_wo: jax.Array,
    B_x: jax.Array,
    B_w1: jax.Array,
    B_b1: jax.Array,
    B_w2: jax.Array,
    B_b2: jax.Array,
    grad_out: jax.Array,
):
    del B_x
    hbm = pl.BlockSpec(memory_space=pl.ANY)
    vmem = pl.BlockSpec(memory_space=pltpu.VMEM)
    sds = jax.ShapeDtypeStruct
    outT, dxT, gwqkv, gwo, gw1, gb1, gw2T, gb2 = pl.pallas_call(
        _kernel,
        in_specs=[hbm, hbm, hbm, hbm, hbm, vmem, hbm, vmem],
        out_specs=[hbm, hbm, hbm, hbm, hbm, vmem, hbm, vmem],
        out_shape=[
            sds((D, S), BF16), sds((D, S), BF16), sds((D, 3 * D), BF16), sds((D, D), BF16),
            sds((D, F), BF16), sds((NF, 1, FC), BF16), sds((D, F), BF16), sds((1, D), BF16),
        ],
        scratch_shapes=[
            pltpu.VMEM((D, S), BF16),
            pltpu.VMEM((DP, S), BF16),
            pltpu.VMEM((D, S), BF16),
            pltpu.VMEM((D, S), BF16),
            pltpu.VMEM((S, DP), BF16),
            pltpu.VMEM((S, DP), BF16),
            pltpu.VMEM((D, 3 * D), BF16),
            pltpu.VMEM((DP, D), BF16),
            pltpu.VMEM((2, DP, FC), BF16),
            pltpu.VMEM((2, D, FC), BF16),
            pltpu.VMEM((2, D, FC), BF16),
            pltpu.VMEM((2, D, FC), BF16),
            pltpu.VMEM((S, FC), BF16),
            pltpu.VMEM((S, FC), BF16),
            pltpu.VMEM((S, FC), F32),
            pltpu.VMEM((D, S), F32),
            pltpu.VMEM((D, S), F32),
            pltpu.VMEM((NT_, 3 * D, LANES), F32),
            pltpu.VMEM((NT_, D, LANES), F32),
            pltpu.VMEM((NT_, D, LANES), F32),
            pltpu.VMEM((NT_, 3 * D, LANES), F32),
            pltpu.VMEM((DP, S), BF16),
            pltpu.VMEM((3 * D, S), BF16),
            pltpu.VMEM((D, S), BF16),
            pltpu.VMEM((D, S), BF16),
            pltpu.VMEM((D, 3 * D), BF16),
            pltpu.VMEM((D, D), BF16),
            pltpu.SemaphoreType.DMA((4,)),
            pltpu.SemaphoreType.DMA((2, 2)),
            pltpu.SemaphoreType.DMA((2, 2)),
        ],
        compiler_params=pltpu.CompilerParams(vmem_limit_bytes=120 * 2**20),
    )(A_x[0].T, grad_out[0].T, A_wqkv, A_wo, B_w1, B_b1.reshape(NF, 1, FC), B_w2.T, B_b2.reshape(1, D))
    return (outT.T[None], dxT.T[None], gwqkv, gwo, gw1, gb1.reshape(F), gw2T.T, gb2.reshape(D))
```

```python
from functools import partial

import jax
import jax.numpy as jnp
from jax import lax
import jax.experimental.pallas as pl
import jax.experimental.pallas.tpu as pltpu

BF16, F32, U32 = jnp.bfloat16, jnp.float32, jnp.uint32

S, D, F = 2048, 576, 4608
DH, WIN, DIL = 18, 8, 2
LANES = 128
TS, FC = 512, 512
NJ, NF = S // TS, F // FC
TPB = TS // LANES
DM = 512
M2 = D // 4
MR = 48
PR = 4 * DH
NP = D // PR
MOVES = [(b, m) for b in range(TPB) for m in range(3) if m < 2 or b > 0]
DP = 5 * LANES
KH = 7 * LANES
EPS = 1e-5
SCALE = DH ** -0.5
C0 = 0.7978845608028654
C1 = C0 * 0.044715

NN = (((1,), (0,)), ((), ()))
NT = (((1,), (1,)), ((), ()))

TA = ({(0, 0): 1, (1, 1): 1}, {(1, 0): 1, (1, 1): 1}, {(0, 0): 1}, {(1, 1): 1},
      {(0, 0): 1, (0, 1): 1}, {(1, 0): 1, (0, 0): -1}, {(0, 1): 1, (1, 1): -1})
TB = ({(0, 0): 1, (1, 1): 1}, {(0, 0): 1}, {(0, 1): 1, (1, 1): -1}, {(1, 0): 1, (0, 0): -1},
      {(1, 1): 1}, {(0, 0): 1, (0, 1): 1}, {(1, 0): 1, (1, 1): 1})
TC = ({(0, 0): 1, (1, 1): 1}, {(1, 0): 1, (1, 1): -1}, {(0, 1): 1, (1, 1): 1}, {(0, 0): 1, (1, 0): 1},
      {(0, 1): 1, (0, 0): -1}, {(1, 1): 1}, {(0, 0): 1})
REM = {1: (1, (0,)), 4: (0, (1,)), 5: (1, (0, 1)), 6: (0, (0, 1))}
ORDER = (6, 5, 0, 1, 2, 3, 4)

ATT_COST = (20, 25, 70, 24, 0)
ATT_SPLIT = (2, 5, 9)
ATT_TILES = (2,)
ATT_SPAN = (0, 125)
ACT_IDLE = (2, 6)
STAGE1_ORDER = (0, 1, 2, 3, 4, 5, 6)
GRAD_FIRST = (0, 1)
DUE_DACT = (80, 111)
DUE_DGRAD_OPERANDS = (1, 111)
OUT_PROJ_AHEAD = (2,)
DUE_FINISH_W1 = (20, 100)
DUE_FINISH_W2 = (160, 209)
DUE_PREP2_W1 = (64, 111)
DUE_PREP2_W2 = (0, 0)
DUE_PREP1 = ((60, 100), (154, 174))
DUE_NORMALIZE = (0, 6)
DUE_SECOND = ((4, 11), (0, 0))
DUE_FIRST = ((9, 10), (0, 0))
DUE_WEIGHTS = ((6, 11), (0, 0))
DUE_LAST_FINISH = ((5, 8), (0, 0))
DUE_DX = (0, 14)
DUE_OUT = (1, 15)


def _dot(a, b, dn=NN):
    return lax.dot_general(a, b, dn, preferred_element_type=F32)


def _pack(lo, hi):
    return pltpu.pack_elementwise([lo, hi], packed_dtype=BF16)


def _unpack(w):
    return [pltpu.unpack_elementwise(w, index=i, packed_dtype=BF16, unpacked_dtype=F32) for i in range(2)]


def _bf(w):
    return pltpu.bitcast(w, BF16)


def _signed_sum(terms):
    terms = sorted(terms, key=lambda t: -t[0])
    acc = terms[0][1]
    for c, v in terms[1:]:
        acc = acc + v if c > 0 else acc - v
    return acc


def _operand(row, get, n):
    return {(p, q): _signed_sum([(c, get(i * n + p, j * n + q)) for (i, j), c in row.items()])
            for p in range(n) for q in range(n)}


def _operands(table, get):
    return [_operand(row, get, 1)[0, 0] for row in table]


def _combine(table, prods):
    return {(i, j): _signed_sum([(row[i, j], prods[r]) for r, row in enumerate(table) if (i, j) in row])
            for i in range(2) for j in range(2)}


def _gelu_pair(x):
    x2 = x * x
    t = jnp.tanh(x * (C0 + C1 * x2))
    a = 1.0 + t
    h = x * a
    return h, a + (h * (1.0 - t)) * (C0 + (3.0 * C1) * x2)


def _colmean(parts):
    return sum(jnp.sum(a, axis=0, keepdims=True) for a in parts) * (1.0 / D)


def _layernorm(parts):
    m = _colmean(parts)
    c = [a - m for a in parts]
    r = lax.rsqrt(_colmean([a * a for a in c]) + EPS)
    return [a * r for a in c], (m, r)


class _Deadlines:
    def __init__(self, never):
        self.never, self.due, self.count = never, {}, 0

    def spread(self, works, token, lo, hi):
        if hi == 0:
            self.due.setdefault(None, []).extend(works)
            return
        for c, work in enumerate(works):
            self.due.setdefault(lo + (hi - lo) * (c + 1) // len(works), []).append((work, token))

    def rest(self):
        for work in self.due.get(None, ()):
            work()

    def lhs(self, w):
        for work, token in self.due.get(self.count, ()):
            work()
            head = jnp.where(self.never, pltpu.bitcast(token(), U32), w[:8, :LANES])
            if w.shape[1] > LANES:
                head = jnp.concatenate([head, w[:8, LANES:]], axis=1)
            w = jnp.concatenate([head, w[8:]], axis=0)
        self.count += 1
        return _bf(w)


def _attention_work(p, j, att, old, tmp, base):
    nd = DH // 2
    moves = MOVES

    def rows(i):
        return pl.ds(p * PR + i, 8, stride=9)

    def tap(a, w):
        b = (a - w) % TPB
        return moves.index((b, (b - a + w) // TPB))

    def slot(n):
        return base + n // 32, pl.ds(n % 32 * 8, 8), slice(None)

    def ver(c, n, i):
        return slot((c * len(moves) + n) * nd + i)

    def coef(c, a, w):
        return slot(2 * len(moves) * nd + (c * TPB + a) * (WIN + 1) + w)

    def masks():
        lane = lax.broadcasted_iota(jnp.int32, (8, LANES), 1)
        return lane, jnp.broadcast_to(j, (8, LANES)) > 0

    def shift(c, i):
        lane, inner = masks()
        src = [att[j * TPB + b, 1 + c, rows(i), :] for b in range(TPB)]
        out = []
        for n, (b, m) in enumerate(moves):
            if m == 0:
                out.append(src[b])
            else:
                r = pltpu.roll(src[b], DIL * m, 1)
                out.append(jnp.where(lane >= DIL * m, r, old[c, n, i]))
                old[c, n, i] = r

        def store():
            for n, v in enumerate(out):
                tmp[ver(c, n, i)] = v
        return store

    def dots(a, c, ws):
        even = (lax.broadcasted_iota(jnp.int32, (8, LANES), 0) & 1) == 0
        x = [att[j * TPB + a, 3 * c, rows(i), :] for i in range(nd)]
        y = {w: [tmp[ver(c, tap(a, w), i)] for i in range(nd)] for w in ws}

        def store():
            for w in ws:
                t = sum((x[i] * y[w][i] for i in range(1, nd)), x[0] * y[w][0])
                tmp[coef(c, a, w)] = t + jnp.where(even, pltpu.roll(t, 7, 0), pltpu.roll(t, 1, 0))
        return store

    def softmax(a):
        lane, inner = masks()
        valid = [inner | (lane >= DIL * moves[tap(a, w)][1]) if moves[tap(a, w)][1] else None for w in range(WIN)]
        lg = [tmp[coef(0, a, w)] * SCALE for w in range(WIN)]
        da = [tmp[coef(1, a, w)] for w in range(WIN)]

        def store():
            masked = [t if ok is None else jnp.where(ok, t, -1e9) for t, ok in zip(lg, valid)]
            top = masked[0]
            for t in masked[1:]:
                top = jnp.maximum(top, t)
            e = [jnp.exp(t - top) for t in masked]
            inv = 1.0 / sum(e[1:], e[0])
            pr = [t * inv for t in e]
            mean = sum((pr[w] * da[w] for w in range(1, WIN)), pr[0] * da[0])
            for w in range(WIN):
                dl = (pr[w] * SCALE) * (da[w] - mean)
                tmp[coef(0, a, w)] = dl if valid[w] is None else jnp.where(valid[w], dl, 0.0)
                tmp[coef(1, a, w)] = pr[w]
            tmp[coef(1, a, WIN)] = sum(jnp.where(ok, 0.0, t) for t, ok in zip(pr, valid) if ok is not None)
        return store

    def scatter(b, c, ids):
        lane, inner = masks()
        before = jnp.maximum(j - 1, 0) * TPB + b
        cf = {(a, w): tmp[coef(c, a, w)] for a in range(TPB) for w in range(WIN) if moves[tap(a, w)][0] == b}
        for i in ids:
            x = [att[j * TPB + a, 3 * c, rows(i), :] for a in range(TPB)]
            by_move = {}
            for (a, w), t in cf.items():
                by_move.setdefault(moves[tap(a, w)][1], []).append(t * x[a])
            acc = sum(by_move[0][1:], by_move[0][0])
            if c == 1 and b == 0:
                lost = sum(tmp[coef(1, a, WIN)] * x[a] for a in range(TPB))
                acc = acc + jnp.where(lane == 0, jnp.sum(lost, axis=1, keepdims=True), 0.0)
            back = None
            for m in sorted(by_move)[1:]:
                r = pltpu.roll(sum(by_move[m][1:], by_move[m][0]), LANES - DIL * m, 1)
                here = lane < LANES - DIL * m
                acc = acc + jnp.where(here, r, 0.0)
                t = jnp.where(here, 0.0, r)
                back = t if back is None else back + t
            att[before, 1 + c, rows(i), :] = att[before, 1 + c, rows(i), :] + jnp.where(inner, back, 0.0)
            att[j * TPB + b, 1 + c, rows(i), :] = acc

    def gather(a, c, ids):
        tiles = range(a, a + ATT_TILES[0]) if a % ATT_TILES[0] == 0 else ()
        cf = {(t, w): tmp[coef(c, t, w)] for t in tiles for w in range(WIN)}
        for i in ids:
            y = {n: tmp[ver(c, n, i)] for n in sorted({tap(t, w) for t, w in cf})}
            for t in tiles:
                att[j * TPB + t, 3 * c, rows(i), :] = sum(
                    (cf[t, w] * y[tap(t, w)] for w in range(1, WIN)), cf[t, 0] * y[tap(t, 0)])

    pairs = [(a, c) for c in range(2) for a in range(TPB)]

    def split(n, size):
        return [range(k, min(k + size, n)) for k in range(0, n, size)]

    return ([(partial(shift, c, i), ATT_COST[0]) for c in range(2) for i in range(nd)]
            + [(partial(dots, *t, ws), ATT_COST[1] * len(ws)) for t in pairs for ws in split(WIN, ATT_SPLIT[0])]
            + [(partial(softmax, a), ATT_COST[2]) for a in range(TPB)]
            + [(partial(scatter, *t, ids), ATT_COST[3] * len(ids)) for t in pairs for ids in split(nd, ATT_SPLIT[1])]
            + [(partial(gather, *t, ids), ATT_COST[4] * len(ids)) for t in pairs for ids in split(nd, ATT_SPLIT[2])])


def _kernel(xT_hbm, gT_hbm, wqkv_hbm, wo_hbm, w1_hbm, b1_ref, w2T_hbm, b2_ref,
            outT_hbm, dxT_hbm, gwqkv_hbm, gwo_hbm, gw1_hbm, gb1_ref, gw2T_hbm, gb2_ref,
            xT, g_in, gT, left, pm, wqkv, wq, wo, woT, att, n_dy, n_out, gb1_acc, stats, g_w1, g_w2, st_w1, st_w2, zs, sem_x, sem_w, sem_out):
    nacc, gacc, stage = (n_dy, n_out), (g_w1, g_w2), (st_w1, st_w2)

    def block(j):
        return pl.ds(pl.multiple_of(j * TS, TS), TS)

    def in_copies(j, n):
        src, dst = ((gT_hbm, g_in), (xT_hbm, xT))[n]
        return pltpu.make_async_copy(src.at[:, block(j)], dst.at[j], sem_x.at[n, j])

    def g_copies(i):
        cols = pl.ds(pl.multiple_of(i * FC, FC), FC)
        return [pltpu.make_async_copy(stage[z].at[i % 2, :, pl.ds(0, M2)], g.at[:, :, cols], sem_out.at[i % 2, z])
                for z, g in enumerate((gw1_hbm, gw2T_hbm))]

    def finish(j, slot, z, c):
        rows = pl.ds(pl.multiple_of(j * MR + 16 * c, 16), 16)
        for k in range(4):
            out = _combine(TB, [gacc[z][slot, 4 * r + k, rows, :] for r in range(7)])
            for (p, q), v in out.items():
                col = (2 * q + k % 2) * LANES
                stage[z][slot, 2 * p + k // 2, rows, col:col + LANES] = v.astype(BF16)
            zero = jnp.where(zs[0] > 0, v, 0.0)
            for r in range(7):
                gacc[z][slot, 4 * r + k, rows, :] = zero

    def reorder(ref, j, forward, dest=None):
        w = pltpu.bitcast(ref[j], U32)
        w = jnp.concatenate([w, jnp.zeros((3 * LANES - D // 2, TS), U32)], axis=0)
        for l in range(3):
            for n in range(TPB):
                pm[0, l, n * LANES:(n + 1) * LANES, :] = w[l * LANES:(l + 1) * LANES, n * LANES:(n + 1) * LANES].T
            for a in range(TPB):
                for e in range(2):
                    spaced, packed = pl.ds(2 * a + e, TS // 8, stride=8), pl.ds(a * LANES + e, TS // 8, stride=2)
                    src, dst = (spaced, packed) if forward else (packed, spaced)
                    pm[1, l, dst, :] = pm[0, l, src, :]
        w = jnp.concatenate([jnp.concatenate([pm[1, l, n * LANES:(n + 1) * LANES, :].T for n in range(TPB)], axis=1)
                             for l in range(3)], axis=0)
        (ref if dest is None else dest)[j] = _bf(w[:D // 2])

    def halves(ref, j, n):
        return _unpack(pltpu.bitcast(ref[j, :, n * LANES:(n + 1) * LANES], U32))

    cp_wo = pltpu.make_async_copy(wo_hbm, wo.at[pl.ds(0, D)], sem_w.at[0])
    cp_wqkv = pltpu.make_async_copy(wqkv_hbm, wqkv, sem_w.at[1])
    for k in range(3):
        zs[k] = 0

    def mlp_phase(a1, a2, b1y, b1g, b2y, b2g, raw, xs, dps, old, tr0, tr1, ys0, ys1, gsum, wqkvT, b1_rows,
                  sem_in, sem_z, *cs):
        tr, ys = (tr0, tr1), (ys0, ys1)
        b1, b2 = (b1y, b1g), (b2y, b2g)
        c_s = (cs[:7], cs[7:])

        def w_copies(i):
            cols = pl.ds(pl.multiple_of(i * FC, FC), FC)
            return [pltpu.make_async_copy(w.at[:, cols], raw.at[i % 2, z], sem_in.at[i % 2, z])
                    for z, w in enumerate((w1_hbm, w2T_hbm))]

        def raw_rows(slot, z, row, lanes):
            return _unpack(pltpu.bitcast(raw[slot, z, pl.ds(pl.multiple_of(row, 16), 16), lanes], U32))

        def prep1(i, j, slot, z):
            half = FC // 2
            for ro in range(0, DM // 2 // NJ, 16):
                o = j * (DM // 2 // NJ) + ro
                blk = {(p, q): raw_rows(slot, z, p * (DM // 2) + o, slice(q * half, (q + 1) * half))
                       for p in range(2) for q in range(2)}
                lo, hi = (_operands(TB, lambda p, q: blk[p, q][e]) for e in range(2))
                for r in range(7):
                    b1[z][slot, r, pl.ds(pl.multiple_of(o // 2, 8), 8), :] = _pack(lo[r], hi[r])
            blk = [raw_rows(slot, z, DM + j * 16, slice(q * half, (q + 1) * half)) for q in range(2)]
            if z == 0:
                first = lax.broadcasted_iota(jnp.int32, (8, half), 0) == 0
                bias = b1_rows[i]
                bias = [jnp.where(first, bias[:, q * half:(q + 1) * half], 0.0) for q in range(2)]
            for r, (_, qs) in REM.items():
                b1[z][slot, r, pl.ds(pl.multiple_of(DM // 4 + j * 8, 8), 8), :] = _pack(
                    *(_signed_sum([(1, blk[q][e]) for q in qs]) for e in range(2)))
                if z == 0:
                    b1[z][slot, r, (DM // 2 + D - DM) // 2:(DM // 2 + D - DM) // 2 + 8, :] = _pack(
                        _signed_sum([(1, bias[q]) for q in qs]), jnp.zeros((8, half), F32))

        def prep2(j, slot, z, c):
            o = jnp.minimum(j * MR, M2 - MR) + 16 * c
            blk = {(p, q): raw_rows(slot, z, p * M2 + o, slice(q * LANES, (q + 1) * LANES))
                   for p in range(4) for q in range(4)}
            for r in range(7):
                lo, hi = (_operand(TB[r], lambda p, q: blk[p, q][e], 2) for e in range(2))
                for p, q in lo:
                    b2[z][slot, r, pl.ds(pl.multiple_of((p * M2 + o) // 2, 8), 8), q * LANES:(q + 1) * LANES] = (
                        _pack(lo[p, q], hi[p, q]))

        def second_operands(z, j, starts):
            h2 = M2 // 2
            for ro in starts:
                blk = [{(p, q): 0.5 * ys[z][e, p, q * h2 + ro:q * h2 + ro + 8, :] for p in range(4) for q in range(4)}
                       for e in range(2)]
                for r in range(7):
                    lo, hi = (_operand(TA[r], lambda p, q: blk[e][p, q], 2) for e in range(2))
                    for p, q in lo:
                        a2[z, j, r, q * h2 + ro:q * h2 + ro + 8, p * LANES:(p + 1) * LANES] = _pack(lo[p, q], hi[p, q])

        def first_operands(z, j):
            h1, t1 = DM // 4, TS // 2

            def wide(e, p, lo, hi):
                return jnp.concatenate([ys[z][e, 2 * p + n, lo:hi, :] for n in range(2)], axis=1)

            ops = [_operands(TA, lambda p, q: wide(e, p, q * h1, (q + 1) * h1)) for e in range(2)]
            pad = lax.broadcasted_iota(jnp.int32, (LANES // 2 - (D - DM) // 2, t1), 0)
            one = jnp.where(pad == 0, 1.0 - z, 0.0)
            rem = [_bf(jnp.concatenate([_pack(wide(0, p, DM // 2, D // 2), wide(1, p, DM // 2, D // 2)),
                                        _pack(one, jnp.zeros_like(one))], axis=0)).T for p in range(2)]
            for r in range(7):
                parts = [_bf(_pack(ops[0][r], ops[1][r])).T]
                if r in REM:
                    parts.append(rem[REM[r][0]])
                w = pltpu.bitcast(jnp.concatenate(parts, axis=1), U32)
                for l in range(w.shape[1] // LANES):
                    tr[z][r, l] = w[:, l * LANES:(l + 1) * LANES]
                    for b in range(t1 // LANES):
                        ev, od = (tr[z][r, l, pl.ds(b * 64 + e, 32, stride=2), :] for e in range(2))
                        a1[z, j, r, b * 64:b * 64 + 32, l * LANES:(l + 1) * LANES] = (ev & 0xFFFF) | (od << 16)
                        a1[z, j, r, b * 64 + 32:b * 64 + 64, l * LANES:(l + 1) * LANES] = (
                            (ev >> 16) | (od & jnp.uint32(0xFFFF0000)))

        in_copies(0, 0).start()
        cp_wo.start()
        for j in range(NJ):
            in_copies(j, 1).start()
            if j + 1 < NJ:
                in_copies(j + 1, 0).start()
        cp_wqkv.start()
        for c in w_copies(0) + w_copies(1):
            c.start()
        zero = n_dy.at[0]
        zero[...] = jnp.zeros(zero.shape, F32)
        clears = [(zero, nacc[z].at[j]) for z in range(2) for j in range(NJ) if z or j]
        for z in range(2):
            for slot in range(2):
                clears.append((zero, gacc[z].at[slot, :, pl.ds(0, M2)]))
                clears.append((zero.at[:, pl.ds(0, MR)], gacc[z].at[slot, :, pl.ds(M2, MR)]))
        clears = [pltpu.make_async_copy(a, b, sem_z.at[n]) for n, (a, b) in enumerate(clears)]
        for n in range(NF):
            b1_rows[n] = b1_ref[n * FC:(n + 1) * FC].astype(F32).reshape(1, FC)
        for c in clears:
            c.start()
        in_copies(0, 0).wait()
        reorder(g_in, 0, True, gT)
        cp_wo.wait()
        pad = lax.broadcasted_iota(jnp.int32, (DP - D, D), 0)
        wo[D:, :] = jnp.where(pad == 0, b2_ref[...].astype(F32).reshape(1, D), 0.0).astype(BF16)

        def pro_g(j, carry_):
            pl.when(j + 1 < NJ)(lambda: in_copies(j + 1, 0).wait())
            in_copies(j, 1).wait()
            reorder(xT, j, True)
            val = _dot(wo[:D, :], gT[j])
            for n in range(TPB):
                att[j * TPB + n, 3, :D, :] = val[:, n * LANES:(n + 1) * LANES]
                att[j * TPB + n, :, D:, :] = jnp.zeros((4, PR, LANES), F32)
            for n in range(TPB):
                xn, first = _layernorm(halves(xT, j, n))
                left[0, j, :, n * LANES:(n + 1) * LANES] = _pack(*xn)
                for k, v in enumerate(first):
                    stats[j * TPB + n, k] = jnp.broadcast_to(v, (8, LANES))
            reorder(g_in, jnp.minimum(j + 1, NJ - 1), True, gT)
            return carry_

        gsum[...] = jnp.zeros(gsum.shape, F32)
        lax.fori_loop(0, NJ, pro_g, 0)
        cp_wqkv.wait()
        for n in range(0, 3 * D, 3 * LANES):
            cols = slice(n, min(n + 3 * LANES, 3 * D))
            wqkvT[n // 2:cols.stop // 2, :] = pltpu.bitcast(wqkv[:, cols].T, U32)
        for c in w_copies(0):
            c.wait()

        def pro_x(j, carry_):
            for z in range(2):
                for slot in range(2):
                    for r in REM:
                        b1[z][slot, r, pl.ds(pl.multiple_of((DM // 2 + D - DM) // 2 + j * 8, 8), 8), :] = (
                            jnp.zeros((8, FC // 2), U32))

            def normalize(n):
                m, r = (stats[j * TPB + n, k, :1, :] for k in range(2))
                y, second = _layernorm([(a - m) * r for a in halves(xT, j, n)])
                for k, v in enumerate(second):
                    stats[j * TPB + n, 2 + k] = jnp.broadcast_to(v, (8, LANES))
                g = halves(gT, j, n)
                for e in range(2):
                    ys[0][e, n] = y[e]
                    ys[1][e, n] = g[e]
                    gsum[e] += g[e]

            plan, zero = _Deadlines(zs[0] > 0), zs[1]
            plan.spread([partial(normalize, n) for n in range(TPB)], lambda: ys[0][zero, 0, :8, :], *DUE_NORMALIZE)
            for z in range(2):
                plan.spread([partial(second_operands, z, j, range(ro, ro + 24, 8)) for ro in range(0, M2 // 2, 24)],
                            lambda: a2[zero, 0, 0, :8, :LANES], *DUE_SECOND[z])
                plan.spread([partial(first_operands, z, j)], lambda: a1[zero, 0, 0, :8, :LANES], *DUE_FIRST[z])
                plan.spread([partial(prep2, j, 0, z, c) for c in range(MR // 16)],
                            lambda z=z: b2[z][zero, 0, :8, :LANES], *DUE_WEIGHTS[z])
                prep1(0, j, 0, z)
            for m in range(0, 3 * D, M2):
                val = _dot(plan.lhs(wqkvT[m // 2:(m + M2) // 2, :]), _bf(left[0, j]))
                for n in range(TPB):
                    att[j * TPB + n, m // D, m % D:m % D + M2, :] = val[:, n * LANES:(n + 1) * LANES]
            plan.rest()
            woT[...] = pltpu.bitcast(wo[...].T, U32)
            for ro in range(0, 2 * MR, 16):
                o = pl.multiple_of(jnp.minimum(j * 2 * MR, 2 * M2 - 2 * MR) + ro, 16)
                rows = [_unpack(pltpu.bitcast(wqkv[pl.ds(p * 2 * M2 + o, 16), :], U32)) for p in range(2)]
                rows = [[jnp.concatenate([a, jnp.zeros((8, 2 * KH - 3 * D), F32)], axis=1) for a in r] for r in rows]
                lo, hi = (_operands(TA, lambda p, q: rows[p][e][:, q * KH:(q + 1) * KH]) for e in range(2))
                for r in range(7):
                    wq[r, pl.ds(pl.multiple_of(o // 2, 8), 8), :] = _pack(lo[r], hi[r])
            return carry_

        lax.fori_loop(0, NJ, pro_x, 0)
        rows = xs.at[pl.ds(0, 3)]
        for n in range(3):
            size = min(LANES, D // 2 - n * LANES)
            if size < LANES:
                rows[n] = jnp.zeros(rows.shape[1:], F32)
            for e in range(2):
                rows[n, pl.ds(e, size, stride=2), :] = gsum[e, n * LANES:n * LANES + size, :]
        total = jnp.concatenate([jnp.sum(rows[n].T, axis=0, keepdims=True) for n in range(3)], axis=1)
        gb2_ref[...] = total[:, :D].reshape(D).astype(BF16)
        for c in clears:
            c.wait()
        gb1_acc[...] = jnp.zeros(gb1_acc.shape, F32)
        for z in range(2):
            stage[z][0, 0, :16, :LANES] = jnp.zeros((16, LANES), BF16)

        t1 = TS // 2
        q_at, h_at, d_at = (0, 14), 28, 36

        def stage2(z, r, j, slot, lhs):
            for grad in ((1, 0) if GRAD_FIRST[z] else (0, 1)):
                v = (_dot(lhs(a2[z, j, r]), _bf(c_s[z][r][...])) if grad
                     else _dot(lhs(b2[z][slot, r]), _bf(c_s[z][r][...]), NT))
                for k in range(4):
                    d, l = divmod(k, 2) if grad else divmod(k, 2)[::-1]
                    t = v[d * M2:(d + 1) * M2, l * LANES:(l + 1) * LANES]
                    if grad:
                        gacc[z][slot, 4 * r + k, :M2] += t
                    else:
                        nacc[z][j, 4 * r + k] += t

        def step(i, j, carry_):
            slot = i % 2
            o_mxu, o_vpu = zs[1], zs[2]
            plan, pending = _Deadlines(zs[0] > 0), []
            lhs = plan.lhs

            def spread(works, token, lo, hi):
                plan.spread(works, token, 14 + (lo - 14) // 7, hi and 14 + (hi - 14) // 7)

            def flush():
                while pending:
                    pending.pop(0)()

            def act(ro, l):
                flush()
                prods = [xs[o_vpu + q_at[0] + 2 * r + l, ro:ro + 16, :] for r in range(7)]

                def store():
                    for (p, q), v in _combine(TC, prods).items():
                        h, dh = _gelu_pair(v)
                        xs[o_vpu + h_at + 4 * p + 2 * q + l, ro:ro + 16, :] = h
                        xs[o_vpu + d_at + 4 * p + 2 * q + l, ro:ro + 16, :] = dh
                pending.append(store)

            def stage1(z, r, side=()):
                k = DM // 2 + (LANES if r in REM else 0)
                v = _dot(lhs(a1[z, j, r, :, :k]), _bf(b1[z][slot, r, :k // 2, :]))
                n = max(1, len(side))
                for c in range(n):
                    lo, hi = c * (t1 // 16) // n * 16, (c + 1) * (t1 // 16) // n * 16
                    for l in range(2 if hi > lo else 0):
                        xs[o_mxu + q_at[z] + 2 * r + l, lo:hi, :] = v[lo:hi, l * LANES:(l + 1) * LANES]
                    if side:
                        side[c]()

            bsum = [jnp.zeros((8, LANES), F32) for _ in range(4)]

            def dact(ro, l):
                prods = [xs[o_mxu + q_at[1] + 2 * r + l, ro:ro + 16, :] for r in range(7)]
                for (p, q), v in _combine(TC, prods).items():
                    dp = v * xs[o_vpu + d_at + 4 * p + 2 * q + l, ro:ro + 16, :]
                    dps[2 * q + l, p * t1 + ro:p * t1 + ro + 16, :] = dp

            def hidden_operand(z, r, starts=range(0, LANES // 2, 8)):
                def get(o, p, q):
                    if z:
                        return xs[o_vpu + h_at + 4 * (p // 2) + q, p % 2 * LANES + o:p % 2 * LANES + o + 8, :]
                    return dps[q, p * LANES + o:p * LANES + o + 8, :]

                for ro in starts:
                    lo, hi = (_operand(TC[r], partial(get, o), 2) for o in (ro, LANES // 2 + ro))
                    if z == 0 and r in (2, 3):
                        for q in range(2):
                            bsum[2 * (3 - r) + q] += (lo[0, q] + hi[0, q]) + (lo[1, q] + hi[1, q])
                    for p, q in lo:
                        c_s[z][r][p * LANES // 2 + ro:p * LANES // 2 + ro + 8, q * LANES:(q + 1) * LANES] = (
                            _pack(lo[p, q], hi[p, q]))

            chunks = [(ro, l) for ro in range(0, t1, 16) for l in range(2)]
            thirds = range(MR // 16)
            nxt = jnp.minimum(i + 1, NF - 1)
            work = _attention_work(i, j, att, old, xs, o_vpu + 44)
            spread([partial(dact, *c) for c in chunks], lambda: dps[o_mxu, :8, :], *DUE_DACT)
            for r in ORDER[:DUE_DGRAD_OPERANDS[0]]:
                spread([partial(hidden_operand, 0, r)], lambda r=r: c_s[0][r][pl.ds(pl.multiple_of(8 * o_mxu, 8), 8), :LANES],
                       DUE_DGRAD_OPERANDS[1], DUE_DGRAD_OPERANDS[1])
            for z, when in ((0, DUE_FINISH_W1), (1, DUE_FINISH_W2)):
                spread([partial(finish, j, 1 - slot, z, c) for c in thirds],
                       lambda z=z: stage[z][o_mxu, 0, :16, :LANES], *when)
            for z, when in ((0, DUE_PREP2_W1), (1, DUE_PREP2_W2)):
                spread([partial(prep2, j, 1 - slot, z, c) for c in thirds],
                       lambda z=z: b2[z][o_mxu, 0, :8, :LANES], *when)
            for z in range(2):
                spread([partial(prep1, nxt, j, 1 - slot, z)], lambda z=z: b1[z][o_mxu, 0, :8, :LANES], *DUE_PREP1[z])

            def paced(thunk):
                flush()
                rest = thunk()
                if rest:
                    pending.append(rest)

            late = [t for t, n in work if not n]
            work = [(t, n) for t, n in work if n]
            slots = 7 * t1 // 16
            side, at, total = [[] for _ in range(slots)], 0, sum(n for _, n in work)
            for thunk, n in work:
                side[min(ATT_SPAN[0] + at * (ATT_SPAN[1] - ATT_SPAN[0]) // total, slots - 1)].append(thunk)
                at += n
            side = [partial(lambda ts: [paced(t) for t in ts], ts) for ts in side]
            for r in range(7):
                stage1(0, STAGE1_ORDER[r], side[r * slots // 7:(r + 1) * slots // 7])
            acts = [partial(act, *c) for c in chunks] + [flush]
            acts += [partial(hidden_operand, 1, r, range(ro, ro + 32, 8))
                     for r in ORDER[:ACT_IDLE[0]] for ro in range(0, LANES // 2, 32)] + [flush] * ACT_IDLE[1]
            for r in range(7):
                stage1(1, STAGE1_ORDER[r], acts[r * len(acts) // 7:(r + 1) * len(acts) // 7])
            for z in (1, 0):
                for r in ORDER:
                    if r not in ORDER[:(DUE_DGRAD_OPERANDS[0], ACT_IDLE[0])[z]]:
                        hidden_operand(z, r)
                    stage2(z, r, j, slot, lhs)
            plan.rest()
            for t in late:
                t()
            gb1_acc[i] += jnp.concatenate(bsum, axis=1)

            return carry_

        def chunk(i, carry_):
            @pl.when(i + 1 < NF)
            def _():
                for c in w_copies(i + 1):
                    c.wait()

            @pl.when(i + 2 < NF)
            def _():
                for c in w_copies(i + 2):
                    c.start()

            @pl.when(i >= 3)
            def _():
                for c in g_copies(i - 3):
                    c.wait()

            for c in range(2):
                for d in range(DH // 2):
                    start = att[0, 1 + c, pl.ds(i * PR + d, 8, stride=9), :][:, 0:1]
                    for n, (_, m) in enumerate(MOVES):
                        if m:
                            old[c, n, d] = jnp.broadcast_to(start, (8, LANES))
            lax.fori_loop(0, NJ, partial(step, i), 0)

            @pl.when(i >= 1)
            def _():
                for c in g_copies(i - 1):
                    c.start()

            return carry_

        lax.fori_loop(0, NF, chunk, 0)
        for c in g_copies(NF - 3):
            c.wait()

    vm = pltpu.VMEM
    kw = DM // 2 + LANES
    pl.run_scoped(
        mlp_phase,
        vm((2, NJ, 7, TS // 4, kw), U32), vm((2, NJ, 7, M2, 2 * LANES), U32),
        *[vm((2, 7, kw // 2, FC // 2), U32)] * 2, *[vm((2, 7, M2, 2 * LANES), U32)] * 2,
        vm((2, 2, D, FC), BF16),
        vm((53, TS // 2, LANES), F32), vm((4, TS, LANES), F32),
        vm((2, 11, DH // 2, 8, LANES), F32),
        *[vm((7, 3, TS // 4, LANES), U32)] * 2, *[vm((2, TPB, D // 2, LANES), F32)] * 2,
        vm((2, D // 2, LANES), F32), vm((3 * D // 2, D), U32), vm((NF, 1, FC), F32),
        pltpu.SemaphoreType.DMA((2, 2)), pltpu.SemaphoreType.DMA((15,)),
        *[vm((LANES, 2 * LANES), U32)] * 14)

    g_at = 3 * D + DP - D

    def out_phase(right, stack, oT, outb, dxb, gw, gw_d, halves_q, sem_o, sem_g):
        gb1_ref[...] = (0.5 * jnp.concatenate([jnp.sum(gb1_acc[n], axis=0, keepdims=True) for n in range(NF)],
                                       axis=1)).reshape(F).astype(BF16)
        ones = lax.broadcasted_iota(jnp.int32, (DP - D, TS), 0) == 0
        oT[D:, :] = jnp.where(ones, 1.0, 0.0).astype(BF16)

        def project(j, carry_):
            for n in range(TPB):
                ln = slice(n * LANES, (n + 1) * LANES)
                oT[:D, ln] = att[j * TPB + n, 3, :D, :].astype(BF16)
                for part in range(3):
                    right[j, part * D:(part + 1) * D, ln] = att[j * TPB + n, part, :D, :].astype(BF16)
            plan, zero = _Deadlines(zs[0] > 0), zs[1]
            for z in range(2):
                plan.spread([partial(finish, j, (NF - 1) % 2, z, c) for c in range(MR // 16)],
                            lambda z=z: stage[z][zero, 0, :16, :LANES], *DUE_LAST_FINISH[z])
            right[j, 3 * D:g_at, :] = jnp.zeros((DP - D, TS), BF16)
            for ro in range(0, KH, 16):
                blk = {(p, q): _unpack(pltpu.bitcast(
                    right[j, p * KH + ro:p * KH + ro + 16, q * TS // 2:(q + 1) * TS // 2], U32))
                    for p in range(2) for q in range(2)}
                lo, hi = (_operands(TB, lambda p, q: blk[p, q][e]) for e in range(2))
                for r in range(7):
                    halves_q[r, ro // 2:ro // 2 + 8, :] = _pack(lo[r], hi[r])

            def attention_out(starts):
                for m in starts:
                    val = _dot(plan.lhs(woT[m // 2:(m + M2) // 2, :]), oT[...])
                    for n in range(TPB):
                        att[j * TPB + n, 3, m:m + M2, :] = val[:, n * LANES:(n + 1) * LANES]

            attention_out(range(0, OUT_PROJ_AHEAD[0] * M2, M2))
            out = _combine(TC, [_dot(plan.lhs(wq[r]), _bf(halves_q[r])) for r in range(7)])
            for (p, q), val in out.items():
                for n in range(2):
                    att[j * TPB + 2 * q + n, 0, p * 2 * M2:(p + 1) * 2 * M2, :] = val[:, n * LANES:(n + 1) * LANES]
            attention_out(range(OUT_PROJ_AHEAD[0] * M2, D, M2))
            plan.rest()
            stack[0, j] = left[0, j]
            stack[1, j] = pltpu.bitcast(oT[:D, :], U32)
            right[j, g_at:g_at + D, :] = gT[j]
            right[j, g_at + D:, :] = jnp.zeros((DP - D, TS), BF16)
            return carry_

        lax.fori_loop(0, NJ, project, 0)
        for c in g_copies(NF - 1):
            c.start()

        def out_copies(j):
            return (pltpu.make_async_copy(dxb.at[j], dxT_hbm.at[:, block(j)], sem_o.at[0, j]),
                    pltpu.make_async_copy(outb.at[j], outT_hbm.at[:, block(j)], sem_o.at[1, j]))

        def gathered(z, j, n, rs):
            kq, lo = divmod(rs.start, M2)
            k = 2 * (n % 2) + kq % 2
            return 0.5 * _signed_sum([(row[n // 2, kq // 2], nacc[z][j, 4 * r + k, lo:lo + rs.stop - rs.start, :])
                                for r, row in enumerate(TA) if (n // 2, kq // 2) in row])

        starts = (0, 4 * LANES, 9 * LANES, g_at)
        copies = [pltpu.make_async_copy(a, b, sem_g.at[c]) for c, (a, b) in enumerate((
            (gw.at[0, :, pl.ds(0, starts[1])], gwqkv_hbm.at[:, pl.ds(0, starts[1])]),
            (gw.at[1], gwqkv_hbm.at[:, pl.ds(starts[1], DP)]),
            (gw_d.at[2], gwqkv_hbm.at[:, pl.ds(starts[2], D)]),
            (gw_d.at[3], gwo_hbm)))]

        def finish_up(c, carry_):
            rows = pl.ds(pl.multiple_of(jnp.where(c < 1, 0, c * DP - LANES), LANES), DP)

            def forward(n):
                ln = slice(n * LANES, (n + 1) * LANES)
                for r in range(0, D, 16):
                    rs = slice(r, r + 16)
                    outb[c, rs, ln] = (xT[c, rs, ln].astype(F32) + att[c * TPB + n, 3, rs, :]
                                       + gathered(1, c, n, rs)).astype(BF16)

            def backward(n):
                ln, t = slice(n * LANES, (n + 1) * LANES), c * TPB + n
                m1, r1, m2, r2 = (jnp.concatenate([stats[t, k]] * 2, axis=0) for k in range(4))
                pieces = [slice(r, r + 16) for r in range(0, D, 16)]

                def normalized(rs):
                    xn = (xT[c, rs, ln].astype(F32) - m1) * r1
                    return xn, (xn - m2) * r2

                s1 = s2 = 0.0
                for rs in pieces:
                    dy = gathered(0, c, n, rs)
                    att[t, 1, rs, :] = dy
                    s1, s2 = s1 + dy, s2 + dy * normalized(rs)[1]
                s1, s2 = _colmean([s1]), _colmean([s2])
                t1 = t2 = 0.0
                for rs in pieces:
                    xn, y = normalized(rs)
                    d = att[t, 0, rs, :] + r2 * (att[t, 1, rs, :] - s1 - y * s2)
                    att[t, 0, rs, :] = d
                    t1, t2 = t1 + d, t2 + d * xn
                t1, t2 = _colmean([t1]), _colmean([t2])
                for rs in pieces:
                    dx = r1 * (att[t, 0, rs, :] - t1 - normalized(rs)[0] * t2)
                    dxb[c, rs, ln] = (gT[c, rs, ln].astype(F32) + dx).astype(BF16)

            plan, zero = _Deadlines(zs[0] > 0), zs[1]
            for buf, fn, when in ((dxb, backward, DUE_DX), (outb, forward, DUE_OUT)):
                plan.spread([partial(fn, n) for n in range(TPB)] + [partial(reorder, buf, c, False)],
                            lambda buf=buf: buf[zero, :16, :LANES], *when)
            for m in range(0, D, M2):
                prods = [_dot(plan.lhs(stack[c // 3, j, m // 2:(m + M2) // 2, :]), right[j, rows, :], NT)
                         for j in range(NJ)]
                grad = sum(prods[1:], prods[0]).astype(BF16)
                gw[c, m:m + M2, :] = grad
                gw_d[c, m:m + M2, :] = grad[:, :D]
            plan.rest()
            for cp in out_copies(c):
                cp.start()
            for k in range(4):
                pl.when(c == k)(copies[k].start)
            return carry_

        lax.fori_loop(0, NJ, finish_up, 0)
        for j in range(NJ):
            for c in out_copies(j):
                c.wait()
        for c in copies + g_copies(NF - 2) + g_copies(NF - 1):
            c.wait()

    pl.run_scoped(
        out_phase,
        vm((NJ, g_at + DP, TS), BF16), vm((2, NJ, D // 2, TS), U32), vm((DP, TS), BF16),
        vm((NJ, D, TS), BF16), vm((NJ, D, TS), BF16), vm((4, D, DP), BF16), vm((4, D, D), BF16), vm((7, KH // 2, TS // 2), U32),
        pltpu.SemaphoreType.DMA((2, NJ)), pltpu.SemaphoreType.DMA((4,)))


@jax.jit
def pallas_parallel_sum__sliding_local_dilated__mixer_channel_mlp__prompt_kernel(
    A_x: jax.Array,
    A_wqkv: jax.Array,
    A_wo: jax.Array,
    B_x: jax.Array,
    B_w1: jax.Array,
    B_b1: jax.Array,
    B_w2: jax.Array,
    B_b2: jax.Array,
    grad_out: jax.Array,
):
    del B_x
    hbm = pl.BlockSpec(memory_space=pl.ANY)
    vmem = pl.BlockSpec(memory_space=pltpu.VMEM)
    sds = jax.ShapeDtypeStruct
    vm = pltpu.VMEM
    outT, dxT, gwqkv, gwo, gw1, gb1, gw2T, gb2 = pl.pallas_call(
        _kernel,
        in_specs=[hbm, hbm, hbm, hbm, hbm, vmem, hbm, vmem],
        out_specs=[hbm, hbm, hbm, hbm, hbm, vmem, hbm, vmem],
        out_shape=[
            sds((D, S), BF16), sds((D, S), BF16), sds((D, 3 * D), BF16), sds((D, D), BF16),
            sds((4, M2, F), BF16), sds((F,), BF16), sds((4, M2, F), BF16), sds((D,), BF16),
        ],
        scratch_shapes=[
            *[vm((NJ, D, TS), BF16)] * 3, vm((1, NJ, D // 2, TS), U32),
            vm((2, 3, TS, LANES), U32), vm((D, 3 * D), BF16), vm((7, M2, KH), U32), vm((DP, D), BF16), vm((D // 2, DP), U32),
            vm((S // LANES, 4, D + PR, LANES), F32),
            vm((NJ, 28, M2, LANES), F32), vm((NJ, 28, M2, LANES), F32),
            vm((NF, 8, FC), F32), vm((S // LANES, 4, 8, LANES), F32), *[vm((2, 28, MR * NJ, LANES), F32)] * 2,
            vm((2, 4, MR * NJ, FC), BF16), vm((2, 4, MR * NJ, FC), BF16),
            pltpu.SMEM((3,), jnp.int32),
            pltpu.SemaphoreType.DMA((2, NJ)), pltpu.SemaphoreType.DMA((2,)), pltpu.SemaphoreType.DMA((2, 2)),
        ],
        compiler_params=pltpu.CompilerParams(vmem_limit_bytes=126 * 2**20),
    )(A_x[0].T, grad_out[0].T, A_wqkv, A_wo, B_w1, B_b1, B_w2.T, B_b2)
    return (outT.T[None], dxT.T[None], gwqkv, gwo, gw1.reshape(D, F), gb1,
            gw2T.reshape(D, F).T, gb2)
```
